```python
import os as _os
_os.environ.setdefault("JAX_PLATFORMS", "cpu")
import jax
import jax.numpy as jnp

def _softmax(x, axis=-1):
    return jax.nn.softmax(x, axis=axis)
def _gelu(x):
    return jax.nn.gelu(x, approximate=True)
def _silu(x):
    return jax.nn.silu(x)
def _sigmoid(x):
    return jax.nn.sigmoid(x)
def _layernorm(x, axis=-1, eps=1e-5):
    m = jnp.mean(x, axis=axis, keepdims=True)
    v = jnp.var(x, axis=axis, keepdims=True)
    return (x - m) / jnp.sqrt(v + eps)
def _scatter_add(tgt, idx, src, axis=0):
    return tgt.at[idx].add(src)
def _segment_sum(src, seg, n):
    return jax.ops.segment_sum(src, seg, n)
class _Rng:
    def __init__(self, key):
        self._k = key
    def _next(self):
        self._k, sub = jax.random.split(self._k)
        return sub
    def normal(self, shape):
        return jax.random.normal(self._next(), shape, dtype=jnp.bfloat16)
    def randint(self, lo, hi, shape):
        return jax.random.randint(self._next(), shape, lo, hi, dtype=jnp.int32)
    def uniform(self, shape, lo=0.0, hi=1.0):
        return jax.random.uniform(self._next(), shape, jnp.bfloat16, lo, hi)
    def permutation(self, n):
        return jax.random.permutation(self._next(), n)


kernel_name = 'interleave_layers__spectral_gfnet__linear_attn_block__prompt'

def setup_inputs():
    _rng = _Rng(jax.random.key(int.from_bytes(__import__("os").urandom(4), "little")))
    _w = (lambda a: (lambda t: t.astype(jnp.bfloat16) if jnp.issubdtype(t.dtype, jnp.floating) else t)(jnp.asarray(a)))
    def _A_setup():
        B, S, D = 1, 2048, 640
        Df = D // 2 + 1
        return {
            "x": _w((lambda *s: _rng.normal(s) * 0.05)(B, S, D)),
            "w_r": _w((lambda *s: _rng.normal(s) * 0.4)(S, Df) * 0.02),
            "w_i": _w((lambda *s: _rng.normal(s) * 0.4)(S, Df) * 0.02),
        }
    _A_in = _A_setup()

    def _B_setup():
        B, S, D = 1, 2048, 640
        return {
            "x": _w((lambda *s: _rng.normal(s) * 0.05)(B, S, D)),
            "wqkv": _w((lambda *s: _rng.normal(s) * 0.05)(D, 3 * D)),
            "wo": _w((lambda *s: _rng.normal(s) * 0.05)(D, D)),
        }
    _B_in = _B_setup()

    return {
        "A_x": _A_in["x"],
        "A_w_r": _A_in["w_r"],
        "A_w_i": _A_in["w_i"],
        "B_x": _B_in["x"],
        "B_wqkv": _B_in["wqkv"],
        "B_wo": _B_in["wo"],
    }

def reference(A_x, A_w_r, A_w_i, B_x, B_wqkv, B_wo):
    def _A_ref(x, w_r, w_i):
        B, S, D = x.shape
        X = (lambda x, axes=(-2,-1): jnp.fft.rfft2(x.astype(jnp.float32), axes=axes))(x, axes=(-2, -1))
        W = w_r + 1j * w_i
        X = X * W
        y = (lambda x, s, axes=(-2,-1): jnp.fft.irfft2(x, s=s, axes=axes).astype(jnp.bfloat16))(X, (S, D), axes=(-2, -1))
        return y

    def _B_ref(x, wqkv, wo):
        B, S, D = x.shape
        H = 32; Dh = D // H
        qkv = (lambda x, *d: x.transpose(*d))((x @ wqkv).reshape(B, S, 3, H, Dh), 2, 0, 3, 1, 4)
        q, k, v = qkv[0], qkv[1], qkv[2]
        phi = lambda t: jnp.where(t > 0, t + 1, jnp.exp(t)) + 1e-6
        pq, pk = phi(q), phi(k)
        kv = jnp.einsum("bhsd,bhse->bhde", pk, v)
        z = jnp.einsum("bhsd->bhd", pk)
        num = jnp.einsum("bhqd,bhde->bhqe", pq, kv)
        den = jnp.einsum("bhqd,bhd->bhq", pq, z)[..., None] + 1e-6
        o = num / den
        return (lambda x, *d: x.transpose(*d))(o, 0, 2, 1, 3).reshape(B, S, D) @ wo

    x = A_x
    x = x + _A_ref(_layernorm(x, axis=-1), A_w_r, A_w_i)
    x = x + _B_ref(_layernorm(x, axis=-1), B_wqkv, B_wo)
    x = x + _A_ref(_layernorm(x, axis=-1), A_w_r, A_w_i)
    x = x + _B_ref(_layernorm(x, axis=-1), B_wqkv, B_wo)
    return x
```

```python
import functools

import jax
import jax.numpy as jnp
import numpy as np
import jax.experimental.pallas as pl
import jax.experimental.pallas.tpu as pltpu

S, D, H = 2048, 640, 32
DH = D // H
DF = D // 2 + 1
R = 32
N2 = S // R
NU = N2 // 8
SUB = 8 * R
LAG = 16
PAD = 24
HEAD, TAIL = 2, 6
GROUPS = (1, 2, 0)
DEFER = (None, 15, 40)
PARTS = ((0, 1024), (1024, S))
KEYS_AT = 44
ROLLED = 3
ROWS = 128
PLAN = (
    "b0 b1 b2 b3 k0 k1 b4 w g0 k2 b5 k3 b6 g1 k4 b7 k5 g2 k6 k7 g3 q0 v q1 m q2 "
    "p0 q3 p1 f0 r0 q4 p2 f1 r1 q5 p3 f2 r2 q6 p4 f3 r3 q7 p5 f4 r4 p6 f5 r5 p7 f6 r6 f7 r7 ",
    "b0 b1 b2 b3 k0 k1 b4 g0 k2 b5 k3 b6 g1 k4 b7 k5 g2 k6 k7 g3 q0 v q1 m q2 "
    "q3 p0 q4 p1 q5 p2 q6 p3 q7 p4 p5 p6 p7")
F32, BF16, U32 = jnp.float32, jnp.bfloat16, jnp.uint32

_C1, _C2 = np.cos(2 * np.pi / 5), np.cos(4 * np.pi / 5)
_S1, _S2 = np.sin(2 * np.pi / 5), np.sin(4 * np.pi / 5)
_RHO = float(_S2 / _S1)
_CD = float((_C1 - _C2) / 2)


_PITCH = N2 + 1
_HALF = (0, R // 2) + tuple(f for f in range(1, R) if (f // (f & -f)) % 4 == 3)


def _words(a):
    a = np.ascontiguousarray(a).astype(np.float32).astype(BF16).view(np.uint16).astype(np.uint32)
    return a[..., 0::2, :] | (a[..., 1::2, :] << 16)


def _group_freqs(g, parity):
    r = g if g % 2 == parity else g + 5
    return r, 10 - r


def _dft_constants():
    fwd, inv = np.zeros((5, 128, 128)), np.zeros((5, 128, 128))
    k = np.concatenate([10 * np.arange(32), 5 + 10 * np.arange(32)])
    th = 2 * np.pi * ((np.arange(128)[:, None] * k[None, :]) % D) / D
    cos, sin = np.cos(th), -np.sin(th)
    sin[:, 0] = np.where(np.arange(128) % 2 == 0, 1.0, -1.0)
    ck = np.full(64, 2.0)
    ck[0] = 1.0
    fwd[0] = np.concatenate([cos, sin], axis=1)
    inv[0] = np.concatenate([cos * ck, sin * ck], axis=1).T / D
    for g in (1, 2):
        for parity in (0, 1):
            k = np.concatenate([r + 10 * np.arange(32) for r in _group_freqs(g, parity)])
            sg = _S1 * (1 - 2 * parity) * np.repeat([1.0, -1.0], 32)[None, :]
            th = 2 * np.pi * ((np.arange(64)[:, None] * k[None, :]) % D) / D
            cos, sin = np.cos(th), np.sin(th)
            f = np.block([[cos, -sin], [-sg * sin, -sg * cos]])
            i = (2.0 / D) * np.block([[cos.T, (sg * sin).T], [-sin.T, (sg * cos).T]])
            fwd[2 * g - 1 + parity] = np.roll(f, 64 * parity, axis=1)
            inv[2 * g - 1 + parity] = np.roll(i, 64 * parity, axis=0)
    return _words(np.concatenate([fwd, inv]))


_DMAT = _dft_constants()


def _sequence_matrices(tfwd, tinv, oct_fwd, oct_inv):
    row = jax.lax.broadcasted_iota(jnp.int32, (8, 2 * N2), 0)
    col = jax.lax.broadcasted_iota(jnp.int32, (8, 2 * N2), 1)

    def unit(k, n):
        angle = (k & (n - 1)).astype(F32) * float(2 * np.pi / n)
        return jnp.cos(angle), jnp.sin(angle)

    mul = lambda a, b: (a[0] * b[0] - a[1] * b[1], a[0] * b[1] + a[1] * b[0])
    pos, imag = (col >> 4) * 8 + (col & 7), (col >> 3) & 1
    fwd = unit(imag * (N2 // 4) - row * pos, N2)
    fwd_rows, fwd_step = unit(-8 * pos, N2), unit(-pos, S)
    inv = [v * (1.0 / S) for v in unit(row * col + jnp.where(col < N2, 0, N2 // 4), N2)]
    inv_rows, inv_step = unit(8 * col, N2), unit(row, S)
    for r in range(0, N2, 8):
        f, i, step = fwd, inv, _twiddle(inv_step, r, S, 1)
        for f1 in range(R // 2 + 1):
            tfwd[f1, r:r + 8], tfwd[f1, N2 + r:N2 + r + 8] = f
            tinv[f1, 2 * r:2 * r + 8], tinv[f1, 2 * r + 8:2 * r + 16] = i
            f, i = mul(f, fwd_step), mul(i, step)
        fwd, inv = mul(fwd, fwd_rows), mul(inv, inv_rows)
    same = (col & 7) == row
    start = inv = [jnp.where(same & (imag == part), 1.0, 0.0) for part in (0, 1)]
    one, four = unit(col >> 4, R), unit(4 * (col >> 4), R)
    for b in range(4):
        f, i, step = start, inv, _twiddle((four[0], -four[1]), b, R, -1)
        for r in range(0, 128, 16):
            oct_fwd[b, r:r + 8], oct_fwd[b, r + 8:r + 16] = f
            oct_inv[b, r:r + 8], oct_inv[b, r + 8:r + 16] = i
            f, i = mul(f, step), mul(i, four)
        inv = mul(inv, one)


def _twiddle(z, num, den, sign):
    re, im = z
    if num == 0:
        return z
    c = float(np.cos(2 * np.pi * num / den))
    s = float(sign * np.sin(2 * np.pi * num / den))
    if (8 * num) % den == 0 and (4 * num) % den != 0:
        if c * s > 0:
            return (re - im) * c, (re + im) * c
        return (re + im) * c, (im - re) * c
    return re * c - im * s, re * s + im * c


def _fft(z, sign, leaf=lambda v: v):
    n = len(z)
    if n == 1:
        return [leaf(z[0])]
    if n == 2:
        (ar, ai), (br, bi) = z
        return [leaf((ar + br, ai + bi)), leaf((ar - br, ai - bi))]
    q = n // 4
    even, odd1, odd3 = [None] * (2 * q), [], []
    for j in range(q):
        (ar, ai), (br, bi), (cr, ci), (dr, di) = z[j], z[j + q], z[j + 2 * q], z[j + 3 * q]
        even[j] = (ar + cr, ai + ci)
        even[j + q] = (br + dr, bi + di)
        ur, ui, vr, vi = ar - cr, ai - ci, br - dr, bi - di
        if sign < 0:
            p, m = (ur + vi, ui - vr), (ur - vi, ui + vr)
        else:
            p, m = (ur - vi, ui + vr), (ur + vi, ui - vr)
        odd1.append(_twiddle(p, j, n, sign))
        odd3.append(_twiddle(m, 3 * j, n, sign))
    out = [None] * n
    out[0::2] = _fft(even, sign, leaf)
    out[1::4] = _fft(odd1, sign, leaf)
    out[3::4] = _fft(odd3, sign, leaf)
    return out


def _fft_dit(get, idx, put=lambda k, v: v):
    n = len(idx)
    if n == 1:
        return [get(idx[0])]
    if n == 2:
        (ar, ai), (br, bi) = get(idx[0]), get(idx[1])
        return [(ar + br, ai + bi), (ar - br, ai - bi)]
    q = n // 4
    even, odd1, odd3 = _fft_dit(get, idx[0::2]), _fft_dit(get, idx[1::4]), _fft_dit(get, idx[3::4])
    out = [None] * n
    for k in range(q):
        (ar, ai), (br, bi) = _twiddle(odd1[k], k, n, -1), _twiddle(odd3[k], 3 * k, n, -1)
        ur, ui, vr, vi = ar + br, ai + bi, ar - br, ai - bi
        (er, ei), (fr, fi) = even[k], even[k + q]
        out[k] = put(k, (er + ur, ei + ui))
        out[k + 2 * q] = put(k + 2 * q, (er - ur, ei - ui))
        out[k + q] = put(k + q, (fr + vi, fi - vr))
        out[k + 3 * q] = put(k + 3 * q, (fr - vi, fi + vr))
    return out


def _leaves(idx):
    return idx if len(idx) <= 2 else _leaves(idx[0::2]) + _leaves(idx[1::4]) + _leaves(idx[3::4])


_ORDER = _leaves(tuple(range(R)))
_SLOT = tuple(_ORDER.index(i) for i in range(R))


class _Lazy:
    def __init__(self, get):
        self.get = get

    def __len__(self):
        return R

    def __getitem__(self, i):
        return self.get(i)


def _rfft(x):
    n = len(x)
    if n == 2:
        return {0: (x[0] + x[1], None), 1: (x[0] - x[1], None)}
    q = n // 4
    odd = _fft([_twiddle((x[j] - x[j + 2 * q], x[j + q] - x[j + 3 * q]), j, n, 1)
                for j in range(q)], 1)
    out = {n - 4 * k - 1: odd[k] for k in range(q)}
    for f, v in _rfft([x[j] + x[j + 2 * q] for j in range(2 * q)]).items():
        out[2 * f] = v
    return out


def _irfft(y, n):
    if n == 2:
        return [y[0][0] + y[1][0], y[0][0] - y[1][0]]
    q = n // 4
    even = _irfft({f // 2: v for f, v in y.items() if f % 2 == 0}, 2 * q)
    odd = _fft([y[n - 4 * k - 1] for k in range(q)], -1)
    odd = [_twiddle(odd[j], j, n, -1) for j in range(q)]
    odd = [v[0] for v in odd] + [v[1] for v in odd]
    return [e + o for e, o in zip(even, odd)] + [e - o for e, o in zip(even, odd)]


def _pair(re, im):
    return jnp.concatenate([re, im], axis=0)


def _bf16(w):
    return pltpu.bitcast(w, BF16)


def _halves(a, b):
    return jnp.where(jax.lax.broadcasted_iota(jnp.int32, a.shape, 1) < 64, a, b)


def _swap(a):
    return pltpu.roll(a, 64, 1)


def _swap_pairs(a):
    lane = jax.lax.broadcasted_iota(jnp.int32, a.shape, 1)
    return jnp.where((lane & 63) == 0, 0.0, _swap(a))


def _skew(t, shift):
    return [_halves(t[i], t[(i - shift) % 5]) for i in range(5)]


def _skew_rows(ref, j):
    return jnp.concatenate(
        [ref[j, 128 * ((i - 3 * b) % 5) + 64 * b:128 * ((i - 3 * b) % 5) + 64 * b + 64, :]
         for i in range(5) for b in range(2)], axis=0)


def _tiles(x):
    return [x[:, 128 * i:128 * (i + 1)] for i in range(5)]


def _center(xs):
    tot = (xs[0] + xs[1]) + (xs[2] + xs[3]) + xs[4]
    mean = jnp.sum(tot, axis=-1, keepdims=True) * (1.0 / D)
    c = [x - mean for x in xs]
    sq = (c[0] * c[0] + c[1] * c[1]) + (c[2] * c[2] + c[3] * c[3]) + c[4] * c[4]
    var = jnp.sum(sq, axis=-1, keepdims=True) * (1.0 / D)
    return c, jax.lax.rsqrt(var + 1e-5)


def _phi(t):
    return jnp.where(t > 0, t + 1.0, jnp.exp(t)) + 1e-6


def _dot(a, b):
    return jax.lax.dot_general(a, b, (((1,), (0,)), ((), ())), preferred_element_type=F32)


def _dot_nt(a, b):
    return jax.lax.dot_general(a, b, (((1,), (1,)), ((), ())), preferred_element_type=F32)


def _quarters(x):
    r, c = x.shape[0] // 2, x.shape[1] // 2
    return x[:r, :c], x[:r, c:], x[r:, :c], x[r:, c:]


def _left_factors(a):
    a11, a12, a21, a22 = _quarters(a)
    return [a11, a11 + a12, a22, a21 + a22, a11 + a22, a12 - a22, a21 - a11]


def _right_factors(b, transposed=False):
    b11, b12, b21, b22 = _quarters(b)
    if transposed:
        b12, b21 = b21, b12
    return [b12 - b22, b22, b21 - b11, b11, b11 + b22, b21 + b22, b11 + b12]


_AS_RIGHT = (5, 2, 6, 0, 4, 3, 1)


def _assemble(m3, m5, m4, m2, m1, m7, m6, transposed=False):
    c12, c21 = m3 + m5, m4 + m2
    if transposed:
        c12, c21 = c21, c12
    return jnp.concatenate([jnp.concatenate([(m4 - m5) + m1 + m7, c12], axis=1),
                            jnp.concatenate([c21, (m3 - m2) + m1 + m6], axis=1)], axis=0)


def _split_rows(a, dtype):
    return ([v.astype(dtype) for v in _left_factors(a[:, 128:])], a[:, :128].astype(dtype),
            a.astype(dtype))


def _split_weights(w):
    return ([v.astype(BF16) for v in _right_factors(w[128:, :512])], w[:128, :512].astype(BF16),
            w[:, 512:].astype(BF16))


def _project(a, w):
    y = _assemble(*[_dot(l, r) for l, r in zip(a[0], w[0])]) + _dot(a[1], w[1])
    return [y[:, i:i + 128] for i in range(0, 512, 128)] + [_dot(a[2], w[2])]


_BANDS = ((0, 144), (120, 264), (240, 400), (376, 520), (496, 640))


def _blocks(fn, n, *tiles):
    outs = [fn(*[t[r:r + n] for t in tiles]) for r in range(0, tiles[0].shape[0], n)]
    return [jnp.concatenate(o, axis=0) for o in zip(*outs)]


def _kernel(x_hbm, wr_hbm, wi_hbm, wqkv_hbm, wo_hbm, dmat_hbm,
            o_hbm,
            io, w_v, wpack, wqkv_v, wo_v, dmat, tfwd, tinv, oct_fwd, oct_inv,
            xs, z1, wfil, w0, wkt, wv, wo, macc,
            sem_in, sem_f, sem_w, sem_out):
    z2 = {}
    direct = {}
    o_cp = [pltpu.make_async_copy(io.at[c], o_hbm.at[:, c], sem_out.at[c]) for c in range(NU)]
    w_cp = [pltpu.make_async_copy(src, dst, sem_w.at[i]) for i, (src, dst) in enumerate((
        (dmat_hbm.at[:5], dmat.at[:5]), (dmat_hbm.at[5:], dmat.at[5:]),
        *[(wqkv_hbm.at[:, D * j:D * (j + 1)], wqkv_v.at[j]) for j in (1, 0, 2)], (wo_hbm, wo_v)))]
    f_cp = [[pltpu.make_async_copy(src.at[:, lo:hi], w_v.at[i, :, lo:hi], sem_f.at[h])
             for i, src in enumerate((wr_hbm, wi_hbm))] for h, (lo, hi) in enumerate(PARTS)]

    def x_copy(u):
        return pltpu.make_async_copy(x_hbm.at[:, u], io.at[u], sem_in.at[u])

    rows8 = lambda y: [y[8 * i:8 * i + 8] for i in _SLOT]
    stack = lambda v: jnp.concatenate([v[i] for i in _ORDER], axis=0)
    hi16 = np.uint32(0xFFFF0000)

    def butterfly(*t):
        a1, a2, b1, b2 = t[1] + t[4], t[2] + t[3], t[1] - t[4], t[2] - t[3]
        sm = a1 + a2
        m = t[0] - 0.25 * sm
        n = (a1 - a2) * _CD
        tot = t[0] + sm
        tot = tot - jnp.sum(tot, axis=-1, keepdims=True) * (5.0 / D)
        sq = 0.4 * (tot * tot) + (1.6 * (m * m + n * n) + (b1 * b1 + b2 * b2))
        rstd = jax.lax.rsqrt(jnp.sum(sq, axis=-1, keepdims=True) * (0.5 / D) + 1e-5)
        out = [tot]
        for re, im in ((m + n, b1 + _RHO * b2), (m - n, _RHO * b1 - b2)):
            a, b = _halves(re, im), _swap(_halves(im, re))
            out += [a + b, a - b]
        return [v * rstd for v in out]

    def feature_dft(lhs, first):
        order = [i for g in GROUPS for i in ((2 * g - 1, 2 * g) if g else (0,))]
        return {i: _dot(lhs[i], _bf16(dmat[first + i])) for i in order}

    def radix8(mat, z):
        y = _dot(mat, jnp.concatenate([_pair(*v) for v in z], axis=0).astype(BF16))
        return [(y[r:r + 8], y[r + 8:r + 16]) for r in range(0, 128, 16)]

    def forward(u, g, y, on_mxu):
        def emit(f1, v):
            if isinstance(u, int):
                direct[g, f1, u] = v
            else:
                z1[g, f1, pl.ds(pl.multiple_of(u * 16, 16), 16), :] = v

        if g:
            e, o = rows8(y[2 * g - 1]), rows8(y[2 * g])

            def put(f1, v):
                emit(f1, _pair(*(v if f1 < R // 2 else v[::-1])))

            get = lambda i: (_halves(e[i], o[i]), _swap(_halves(o[i], e[i])))
            if on_mxu:
                part = [radix8(oct_fwd[b], [get(i) for i in range(b, R, 4)]) for b in range(4)]
                for c in range(8):
                    for d, v in enumerate(_fft([p[c] for p in part], -1)):
                        put(c + 8 * d, v)
            else:
                _fft_dit(get, tuple(range(R)), put)
            return
        for f1, (p, q) in _rfft(rows8(y[0])).items():
            if q is None:
                z = p, _swap_pairs(p)
            elif f1 < R // 2:
                z = p - _swap_pairs(q), _swap_pairs(p) + q
            else:
                z = p + _swap_pairs(q), _swap_pairs(p) - q
            emit(min(f1, R - f1), _pair(*z))

    def filtered(g, f1):
        z = [direct[g, f1, u] if (g, f1, u) in direct else z1[g, f1, 16 * u:16 * u + 16, :]
             for u in range(NU)]
        y = _dot(tfwd[min(f1, R - f1)], jnp.concatenate(z, axis=0).astype(BF16))
        if g == 0:
            w_re, w_im = w0[f1, 0], w0[f1, 1]
        else:
            w = wfil[g, pl.ds(f1 * _PITCH, N2), :]
            w_re, w_im = pltpu.bitcast(w << 16, F32), pltpu.bitcast(w & hi16, F32)
        yr, yi = y[:N2], y[N2:]
        if g and f1 >= R // 2:
            y = [yr * w_re + yi * w_im, yi * w_re - yr * w_im]
        else:
            y = [yr * w_re - yi * w_im, yi * w_re + yr * w_im]
        return jnp.concatenate(y, axis=0).astype(BF16)

    def inverse(u, g, on_mxu):
        ld = lambda f1: (z2[g, f1][16 * u:16 * u + 8], z2[g, f1][16 * u + 8:16 * u + 16])
        if g == 0:
            z = {}
            for f1 in _HALF:
                re, im = ld(min(f1, R - f1))
                z[f1] = (re + _swap_pairs(im), None if f1 % (R // 2) == 0 else
                         im - _swap_pairs(re) if f1 < R // 2 else _swap_pairs(re) - im)
            return [stack(_irfft(z, R))]

        def split(v):
            im = _swap(v[1])
            return _halves(v[0], im), _halves(im, v[0])

        get = lambda f1: ld(f1)[::1 if f1 < R // 2 else -1]
        if on_mxu:
            part = [_fft([get(f1) for f1 in range(c, R, 8)], 1) for c in range(8)]
            part = [radix8(oct_inv[b], [p[b] for p in part]) for b in range(4)]
            z = [split(part[i % 4][i // 4]) for i in range(R)]
        else:
            z = _fft(_Lazy(get), 1, split)
        return [stack(v) for v in zip(*z)]

    def recombine(p0, pe1, po1, pe2, po2, *x):
        a1, b1, a2, b2 = pe1 + po1, _swap(pe1 - po1), pe2 + po2, _swap(pe2 - po2)
        p1, j1, p2, j2 = _halves(a1, b1), _halves(b1, a1), _halves(a2, b2), _halves(b2, a2)
        sm = p1 + p2
        m = p0 - 0.25 * sm
        n = (p1 - p2) * _CD
        u1, u2 = m + n, m - n
        e1, e2 = j1 + _RHO * j2, _RHO * j1 - j2
        x = [a + b for a, b in zip(x, (p0 + sm, u1 - e1, u2 - e2, u2 + e2, u1 + e1))]
        t, rstd = _center(x)
        return jnp.concatenate(x, axis=1), jnp.concatenate([v * rstd for v in t], axis=1)

    def backward(u, parts):
        parts = [parts.get((u, g)) or inverse(u, g, u < HEAD) for g in range(3)]
        p = feature_dft(parts[0] + parts[1] + parts[2], 5)
        xs[u], n = _blocks(recombine, ROWS, *[p[i] for i in range(5)], *_tiles(xs[u]))
        return _split_rows(n, BF16)

    def keys(n, w):
        return _dot_nt(wkt[:, :128], n[1]) + _assemble(
            *[_dot_nt(r, l) for l, r in zip(n[0], w)], transposed=True)

    def gram_update(p, n, acc):
        left = [_left_factors(v) for v in p]
        new = [_dot(left[0][i], n[0][0][j]) + _dot(left[1][i], n[1][0][j])
               for i, j in enumerate(_AS_RIGHT)]
        new.append(_dot(p[0], n[0][1]) + _dot(p[1], n[1][1]))
        new.append(jnp.concatenate([left[0][i] + left[1][i] for i in (1, 3)], axis=0))
        return [a + b for a, b in zip(acc, new)] if acc else new

    def by_head(i):
        sub = jax.lax.broadcasted_iota(jnp.int32, (8, 128), 0)
        out = []
        for d in range(DH):
            for h in range(0, H, 8):
                ld = lambda r: macc[i, pl.ds(PAD + DH * h + r, 8, stride=DH + 1), :]
                out.append(ld(d) if d + 8 <= DH else jnp.where(sub < DH - d, ld(d), ld(d - DH)))
        return jnp.concatenate(out, axis=0)

    def key_sums(z):
        macc[5, PAD:PAD + D] = z
        return _tiles(jnp.sum(by_head(5).T, axis=0, keepdims=True))

    def values(gram):
        out = []
        for j, (lo, hi) in enumerate(_BANDS):
            kv = _dot(gram[lo:hi], _bf16(wv[:, 128 * j:128 * (j + 1)]))
            col = 128 * j + jax.lax.broadcasted_iota(jnp.int32, (1, 128), 1)
            rel = lo + jax.lax.broadcasted_iota(jnp.int32, kv.shape, 0) - (col // DH) * DH
            out.append(jnp.where((rel >= 0) & (rel < DH), kv, 0.0))
        return out

    def mixer(kv):
        done = 0
        for j, (lo, hi) in enumerate(_BANDS):
            mj = _tiles(_dot(kv[j], _bf16(wo[64 * j:64 * (j + 1), :])))
            for i in range(5):
                if done > lo:
                    macc[i, PAD + lo:PAD + done, :] += mj[i][:done - lo]
                macc[i, PAD + done:PAD + hi, :] = mj[i][done - lo:]
            done = hi
        return _split_weights(jnp.concatenate([by_head(i) for i in range(5)], axis=1))

    def normalize(zt, *q):
        pq = [_phi(v) for v in q]
        den = (pq[0] * zt[0] + pq[1] * zt[1]) + (pq[2] * zt[2] + pq[3] * zt[3]) + pq[4] * zt[4]
        den = den + pltpu.roll(den, 64, 1)
        den = den + pltpu.roll(den, 32, 1) + 1e-6
        inv = 1.0 / den
        return [jnp.concatenate([v * inv for v in pq], axis=1)]

    def write(u, x):
        y = jnp.concatenate(_skew(x, -3), axis=1)
        for r in range(R):
            io[u, _ORDER[r]] = y[8 * r:8 * r + 8].astype(BF16)
        o_cp[u].start()

    def filters(g, h):
        for t in range(PARTS[h][0] // 128, PARTS[h][1] // 128):
            col = slice(128 * t, 128 * (t + 1))
            if g == GROUPS[0]:
                re, im = [pltpu.bitcast(w_v[i, :DF - 1, col], U32) for i in (0, 1)]
                wpack[0, t, :D // 4] = (re & np.uint32(0xFFFF)) | (im << 16)
                wpack[1, t, :D // 4] = (re >> 16) | (im & hi16)
            freqs = lambda r: wpack[r % 2, t, pl.ds(r // 2, 32, stride=5), :]
            if g:
                blk = [freqs(r) for parity in (0, 1) for r in _group_freqs(g, parity)]
            else:
                re, im = [pltpu.bitcast(w_v[i, DF - 1:, col].astype(F32), U32) for i in (0, 1)]
                first_row = jax.lax.broadcasted_iota(jnp.int32, (32, 128), 0) == 0
                a, b = freqs(0), freqs(5)
                blk = [a, b, jnp.where(first_row, jnp.broadcast_to((re >> 16) | im, a.shape), a), b]
            blk = pltpu.bitcast(pltpu.bitcast(jnp.concatenate(blk, axis=0), F32).T, U32)
            for i in range(128 // R):
                f2 = t * (128 // R) + i
                lo, hi = blk[R * i:R * i + R // 2], blk[R * i + R // 2:R * (i + 1)]
                wfil[g, pl.ds(f2, R // 2, stride=_PITCH), :] = lo
                wfil[g, pl.ds(R // 2 * _PITCH + N2 - 1 - f2, R // 2, stride=_PITCH), :] = hi
                if g == 0:
                    wfil[0, pl.ds(R * _PITCH + (N2 - f2) % N2, 1), :] = lo[:1]
                    wfil[1, pl.ds(R * _PITCH + f2, 1), :] = hi[:1]

    def real_filters():
        real = (jax.lax.broadcasted_iota(jnp.int32, (N2, 128), 1) & 63) == 0
        for f1 in range(R // 2 + 1):
            pos = wfil[0, pl.ds(f1 * _PITCH, N2), :] if f1 < R // 2 else wfil[1, R * _PITCH:, :]
            neg = wfil[0, pl.ds((R - f1) * _PITCH, N2), :]
            for i, (a, b) in enumerate((
                    (pltpu.bitcast(pos << 16, F32), pltpu.bitcast(neg << 16, F32)),
                    (pltpu.bitcast(pos & hi16, F32), -pltpu.bitcast(neg & hi16, F32)))):
                w = jnp.where(real, a + b, _halves(a, b))
                w0[f1, i] = w if f1 % (R // 2) else 0.5 * w

    def key_weights():
        w_cp[1].wait()
        w_cp[2].wait()
        for cp in w_cp[3:]:
            cp.start()
        wkt[...] = _skew_rows(wqkv_v, 1).T.astype(F32)
        return _right_factors(wkt[:, 128:], transposed=True)

    def value_weights():
        for cp in w_cp[3:]:
            cp.wait()
        wv[...] = pltpu.bitcast(_skew_rows(wqkv_v, 2), U32)
        wo[...] = jnp.concatenate(_skew(_tiles(pltpu.bitcast(wo_v[...], U32)), 3), axis=1)

    def query_weights():
        qt = _tiles(_skew_rows(wqkv_v, 0).T.astype(F32))
        for i in range(5):
            macc[i, PAD:PAD + D] = qt[i]
        return _split_weights(jnp.concatenate([by_head(i).T for i in range(5)], axis=0))

    for cp in [x_copy(u) for u in range(3)] + w_cp[:1]:
        cp.start()
    _sequence_matrices(tfwd, tinv, oct_fwd, oct_inv)
    for i in range(6):
        macc[i, :PAD] = jnp.zeros((PAD, 128), F32)
        macc[i, PAD + D:] = jnp.zeros((32, 128), F32)

    def load(u):
        t = _skew(_tiles(stack([io[u, i].astype(F32) for i in range(R)])), 3)
        xs[u] = jnp.concatenate(t, axis=1)
        return _blocks(butterfly, 2 * ROWS, *t)

    def keep(lhs):
        for i in range(5):
            macc[i, :SUB, :] = lhs[i]

    kept = lambda: [macc[i, :SUB, :] for i in range(5)]
    x_copy(0).wait()
    for cp in [x_copy(u) for u in range(3, NU)]:
        cp.start()
    keep(load(0))
    w_cp[0].wait()

    def first(u, carry):
        x_copy(u + 1).wait()
        for i, cps in enumerate(f_cp):
            @pl.when(u == i)
            def _():
                for cp in cps:
                    cp.start()
        lhs = kept()
        new = load(u + 1)
        y = feature_dft(lhs, 0)
        for g in range(3):
            forward(u, g, y, True)
        keep(new)
        return carry

    jax.lax.fori_loop(0, ROLLED, first, 0)
    for u in range(ROLLED, NU - 1):
        first(u, 0)
    y = feature_dft(kept(), 0)
    for g in range(3):
        forward(NU - 1, g, y, True)

    for cp in f_cp[0]:
        cp.wait()
    for g in GROUPS:
        filters(g, 0)
    for cp in f_cp[1]:
        cp.wait()
    for cp in w_cp[1:3]:
        cp.start()
    for g in GROUPS:
        filters(g, 1)
    real_filters()

    spectra = []
    slots = [(g, f1) for g in GROUPS for f1 in range(R if g else R // 2 + 1)]
    for layer in range(2):
        ys, early = [], {}
        for i in range(len(slots) + LAG):
            if i < len(slots):
                ys.append(filtered(*slots[i]))
            if i >= LAG:
                g, f1 = slots[i - LAG]
                z2[g, f1] = _dot(tinv[min(f1, R - f1)], ys[i - LAG])
                if f1 == 7 and g != GROUPS[0]:
                    done = GROUPS[GROUPS.index(g) - 1]
                    early.update({(u, done): inverse(u, done, True) for u in range(HEAD)})
            if layer == 0 and i == KEYS_AT:
                wk = key_weights()
            if layer and i in DEFER:
                forward(NU - 1, GROUPS[DEFER.index(i)], spectra[NU - 1], True)
        xn, pk, q, lhs, gram = [], [], [], [], None
        for op in PLAN[layer].split():
            u = int(op[1:] or 0)
            if op[0] == "b":
                xn.append(backward(u, early))
            elif op[0] == "k":
                pk.append(_phi(keys(xn[u], wk)))
            elif op[0] == "w":
                value_weights()
                wq = query_weights()
            elif op[0] == "g":
                gram = gram_update(pk[2 * u:2 * u + 2], xn[2 * u:2 * u + 2], gram)
            elif op[0] == "q":
                q.append(_project(xn[u], wq))
            elif op[0] == "v":
                kv = values(jnp.concatenate([gram[7], _assemble(*gram[:7])], axis=1))
                z = key_sums(gram[8])
            elif op[0] == "m":
                mix = mixer(kv)
            elif op[0] == "p":
                o, = _blocks(functools.partial(normalize, z), ROWS, *q[u])
                x = [a + b for a, b in zip(_tiles(xs[u]), _project(_split_rows(o, F32), mix))]
                if layer == 0:
                    xs[u] = jnp.concatenate(x, axis=1)
                    lhs.append(_blocks(butterfly, ROWS, *x))
                else:
                    write(u, x)
            elif op[0] == "f":
                spectra.append(feature_dft(lhs[u], 0))
            else:
                for g in GROUPS[:1 if u == NU - 1 else 3]:
                    forward(u, g, spectra[u], u >= TAIL)
    for cp in o_cp:
        cp.wait()


@jax.jit
def pallas_interleave_layers__spectral_gfnet__linear_attn_block__prompt_kernel(
    A_x: jax.Array,
    A_w_r: jax.Array,
    A_w_i: jax.Array,
    B_x: jax.Array,
    B_wqkv: jax.Array,
    B_wo: jax.Array,
):
    del B_x
    vmem = pltpu.VMEM
    hbm = pl.BlockSpec(memory_space=pltpu.MemorySpace.HBM)
    out = pl.pallas_call(
        _kernel,
        out_shape=jax.ShapeDtypeStruct((R, NU, 8, D), BF16),
        in_specs=[hbm] * 6,
        out_specs=hbm,
        scratch_shapes=[
            vmem((NU, R, 8, D), BF16),
            vmem((2, DF, S), BF16),
            vmem((2, S // 128, D // 4 + 8, 128), U32),
            vmem((3, D, D), BF16),
            vmem((D, D), BF16),
            vmem(_DMAT.shape, U32),
            vmem((R // 2 + 1, 2 * N2, 2 * N2), F32),
            vmem((R // 2 + 1, 2 * N2, 2 * N2), F32),
            vmem((4, 128, 128), F32),
            vmem((4, 128, 128), F32),
            vmem((NU, SUB, D), F32),
            vmem((3, R, 2 * N2, 128), F32),
            vmem((3, R * _PITCH + N2, 128), U32),
            vmem((R // 2 + 1, 2, N2, 128), F32),
            vmem((D, D), F32),
            vmem((D // 2, D), U32),
            vmem((D // 2, D), U32),
            vmem((6, PAD + D + 32, 128), F32),
            pltpu.SemaphoreType.DMA((NU,)),
            pltpu.SemaphoreType.DMA((2,)),
            pltpu.SemaphoreType.DMA((6,)),
            pltpu.SemaphoreType.DMA((NU,)),
        ],
        compiler_params=pltpu.CompilerParams(
            vmem_limit_bytes=100 * 1024 * 1024, flags={"XLA_TPU_FORCE_LP_LLO_SCHEDULER": True}),
    )(A_x.reshape(R, NU, 8, D), A_w_r.T, A_w_i.T, B_wqkv, B_wo, _DMAT)
    return out.reshape(1, S, D)
```
